```python
import os as _os
_os.environ.setdefault("JAX_PLATFORMS", "cpu")
import jax
import jax.numpy as jnp

def _softmax(x, axis=-1):
    return jax.nn.softmax(x, axis=axis)
def _gelu(x):
    return jax.nn.gelu(x, approximate=True)
def _silu(x):
    return jax.nn.silu(x)
def _sigmoid(x):
    return jax.nn.sigmoid(x)
def _layernorm(x, axis=-1, eps=1e-5):
    m = jnp.mean(x, axis=axis, keepdims=True)
    v = jnp.var(x, axis=axis, keepdims=True)
    return (x - m) / jnp.sqrt(v + eps)
def _scatter_add(tgt, idx, src, axis=0):
    return tgt.at[idx].add(src)
def _segment_sum(src, seg, n):
    return jax.ops.segment_sum(src, seg, n)
class _Rng:
    def __init__(self, key):
        self._k = key
    def _next(self):
        self._k, sub = jax.random.split(self._k)
        return sub
    def normal(self, shape):
        return jax.random.normal(self._next(), shape, dtype=jnp.bfloat16)
    def randint(self, lo, hi, shape):
        return jax.random.randint(self._next(), shape, lo, hi, dtype=jnp.int32)
    def uniform(self, shape, lo=0.0, hi=1.0):
        return jax.random.uniform(self._next(), shape, jnp.bfloat16, lo, hi)
    def permutation(self, n):
        return jax.random.permutation(self._next(), n)


kernel_name = 'interleave_layers__gqa_block_cached__dense_activation_mish__decode'

def setup_inputs():
    _rng = _Rng(jax.random.key(int.from_bytes(__import__("os").urandom(4), "little")))
    _w = (lambda a: (lambda t: t.astype(jnp.bfloat16) if jnp.issubdtype(t.dtype, jnp.floating) else t)(jnp.asarray(a)))
    def _A_setup():
        B, Sq, D = 1, 1, 512
        Hq, Hkv, Sk, Dh = 32, 8, 65536, 128
        assert Hq % Hkv == 0, (Hq, Hkv)
        return {
            "x": _w((lambda *s: _rng.normal(s) * 0.05)(B, Sq, D)),
            "k_cache": _w((lambda *s: _rng.normal(s) * 1.6)(B, Hkv, Sk, Dh)),
            "v_cache": _w((lambda *s: _rng.normal(s) * 1.6)(B, Hkv, Sk, Dh)),
            "wq": _w((lambda *s: _rng.normal(s) * 1.6)(D, Hq * Dh) * (D ** -0.5)),
            "wo": _w((lambda *s: _rng.normal(s) * 1.6)(Hq * Dh, D) * ((Hq * Dh) ** -0.5)),
        }
    _A_in = _A_setup()

    def _B_setup():
        B, S, D, F = 1, 1, 512, 1792
        return {
            "x": _w((lambda *s: _rng.normal(s) * 0.05)(B, S, D)),
            "w1": _w((lambda *s: _rng.normal(s) * 0.8)(D, F) * (D ** -0.5)),
            "b1": _w((lambda *s: _rng.normal(s) * 0.8)(F)),
            "w2": _w((lambda *s: _rng.normal(s) * 0.8)(F, D) * (F ** -0.5)),
        }
    _B_in = _B_setup()

    return {
        "A_x": _A_in["x"],
        "A_k_cache": _A_in["k_cache"],
        "A_v_cache": _A_in["v_cache"],
        "A_wq": _A_in["wq"],
        "A_wo": _A_in["wo"],
        "B_x": _B_in["x"],
        "B_w1": _B_in["w1"],
        "B_b1": _B_in["b1"],
        "B_w2": _B_in["w2"],
    }

def reference(A_x, A_k_cache, A_v_cache, A_wq, A_wo, B_x, B_w1, B_b1, B_w2):
    def _A_ref(x, k_cache, v_cache, wq, wo):
        B, Sq, D = x.shape
        Hq, Dh = 32, 128
        Hkv = k_cache.shape[1]
        rep = Hq // Hkv
        q = (lambda x, *d: x.transpose(*d))((x @ wq).reshape(B, Sq, Hq, Dh), 0, 2, 1, 3)
        k = jnp.repeat(k_cache, rep, axis=1)
        v = jnp.repeat(v_cache, rep, axis=1)
        scores = jnp.einsum("bhqd,bhkd->bhqk", q, k) * (Dh ** -0.5)
        p = _softmax(scores, axis=-1)
        o = jnp.einsum("bhqk,bhkd->bhqd", p, v)
        return (lambda x, *d: x.transpose(*d))(o, 0, 2, 1, 3).reshape(B, Sq, Hq * Dh) @ wo

    def _B_ref(x, w1, b1, w2):
        h = jnp.einsum("bsd,df->bsf", x, w1) + b1
        sp = jnp.log1p(jnp.exp(-jnp.abs(h))) + jnp.where(h > 0, h, jnp.zeros_like(h))
        act = h * jnp.tanh(sp)
        return jnp.einsum("bsf,fd->bsd", act, w2)

    x = A_x
    x = x + _A_ref(_layernorm(x, axis=-1), A_k_cache, A_v_cache, A_wq, A_wo)
    x = x + _B_ref(_layernorm(x, axis=-1), B_w1, B_b1, B_w2)
    x = x + _A_ref(_layernorm(x, axis=-1), A_k_cache, A_v_cache, A_wq, A_wo)
    x = x + _B_ref(_layernorm(x, axis=-1), B_w1, B_b1, B_w2)
    return x
```

```python
import jax
import jax.numpy as jnp
from jax import lax
import jax.experimental.pallas as pl
import jax.experimental.pallas.tpu as pltpu

BK = 4096
NRING = 4
KDEPTH = 4
LN_EPS = 1e-5
LOG2E = 1.4426950408889634


def _layernorm(x):
    m = jnp.mean(x, axis=-1, keepdims=True)
    d = x - m
    v = jnp.mean(d * d, axis=-1, keepdims=True)
    return d * lax.rsqrt(v + LN_EPS)


def _kernel(x_hbm, k_hbm, v_hbm, wq_hbm, wo_hbm, w1_hbm, b1_hbm, w2_hbm, o_ref,
            kv, wq_s, wo_s, w1_s, w2_s, x_s, b1_s, ring_sem, k_sem, wq_sem, w_sem,
            *, hkv, nb, ncache_heads):
    nstep = hkv * nb
    ncache = ncache_heads * nb
    njobs = ncache + 2 * (nstep - ncache)
    d_model = x_s.shape[-1]
    dh = kv.shape[-1]
    rep = wq_s.shape[-1] // dh
    scale = LOG2E * dh ** -0.5

    def blk(hbm, t):
        return hbm.at[0, t // nb, pl.ds(pl.multiple_of((t % nb) * BK, BK), BK)]

    def kcache_copy(t):
        return pltpu.make_async_copy(blk(k_hbm, t), kv.at[t], k_sem.at[t % KDEPTH])

    def ring_start(n):
        slot = ncache + n % NRING
        r = n % njobs
        u = r - ncache

        @pl.when(u < 0)
        def _():
            pltpu.make_async_copy(blk(v_hbm, r), kv.at[slot], ring_sem.at[n % NRING]).start()

        @pl.when(jnp.logical_and(u >= 0, u % 2 == 0))
        def _():
            pltpu.make_async_copy(blk(k_hbm, ncache + u // 2), kv.at[slot],
                                  ring_sem.at[n % NRING]).start()

        @pl.when(jnp.logical_and(u >= 0, u % 2 == 1))
        def _():
            pltpu.make_async_copy(blk(v_hbm, ncache + u // 2), kv.at[slot],
                                  ring_sem.at[n % NRING]).start()

    def ring_wait(n):
        pltpu.make_async_copy(blk(v_hbm, 0), kv.at[ncache + n % NRING],
                              ring_sem.at[n % NRING]).wait()

    def wq_copy(h):
        return pltpu.make_async_copy(wq_hbm.at[:, pl.ds(h * rep * dh, rep * dh)],
                                     wq_s.at[h], wq_sem.at[h])

    x_cp = pltpu.make_async_copy(x_hbm.at[0], x_s, w_sem.at[0])
    b1_cp = pltpu.make_async_copy(b1_hbm, b1_s, w_sem.at[1])
    wo_cp = pltpu.make_async_copy(wo_hbm, wo_s, w_sem.at[2])
    w1_cp = pltpu.make_async_copy(w1_hbm, w1_s, w_sem.at[3])
    w2_cp = pltpu.make_async_copy(w2_hbm, w2_s, w_sem.at[4])

    x_cp.start()
    wq_copy(0).start()
    for t in range(max(NRING, KDEPTH)):
        if t < KDEPTH:
            kcache_copy(t).start()
        if t < NRING:
            ring_start(t)
    for h in range(1, hkv):
        wq_copy(h).start()
    b1_cp.start()
    wo_cp.start()
    w1_cp.start()
    w2_cp.start()

    row = lax.broadcasted_iota(jnp.int32, (8, dh), 0)

    def attention(p, xn):
        xn_b = xn.astype(jnp.bfloat16)

        def head(h, y):
            if p == 0:
                wq_copy(h).wait()
            qf = jnp.dot(xn_b, wq_s[h], preferred_element_type=jnp.float32)
            q = jnp.zeros((8, dh), jnp.float32)
            for r in range(rep):
                q = jnp.where(row == r, qf[:, r * dh:(r + 1) * dh], q)
            q = q.astype(jnp.bfloat16)
            streamed = h >= ncache_heads

            def step(j, carry):
                m, l, acc = carry
                t = h * nb + j
                n_k = p * njobs + ncache + 2 * (t - ncache)
                n_v = jnp.where(streamed, n_k + 1, p * njobs + t)
                kslot = jnp.where(streamed, ncache + n_k % NRING, t)

                @pl.when(streamed)
                def _():
                    ring_wait(n_k)

                if p == 0:
                    @pl.when(jnp.logical_not(streamed))
                    def _():
                        kcache_copy(t).wait()

                s = lax.dot_general(q, kv[kslot], (((1,), (1,)), ((), ())),
                                    preferred_element_type=jnp.float32)
                m_new = jnp.maximum(m, jnp.max(s, axis=-1, keepdims=True))
                alpha = jnp.exp2((m - m_new) * scale)
                pr = jnp.exp2((s - m_new) * scale)
                l = alpha * l + jnp.sum(pr, axis=-1, keepdims=True)

                @pl.when(jnp.logical_and(streamed, n_k + NRING < 2 * njobs))
                def _():
                    ring_start(n_k + NRING)

                if p == 0:
                    @pl.when(t + KDEPTH < ncache)
                    def _():
                        kcache_copy(t + KDEPTH).start()

                ring_wait(n_v)
                pv = jnp.dot(pr.astype(jnp.bfloat16), kv[ncache + n_v % NRING],
                             preferred_element_type=jnp.float32)
                acc = alpha * acc + pv

                @pl.when(n_v + NRING < 2 * njobs)
                def _():
                    ring_start(n_v + NRING)

                return m_new, l, acc

            init = (jnp.full((8, 1), -1e30, jnp.float32), jnp.zeros((8, 1), jnp.float32),
                    jnp.zeros((8, dh), jnp.float32))
            _, l, acc = lax.fori_loop(0, nb, step, init)
            o = acc / l
            lhs = jnp.concatenate([jnp.where(row == r, o, 0.0) for r in range(rep)], axis=1)
            wo_h = wo_s[pl.ds(pl.multiple_of(h * rep * dh, rep * dh), rep * dh), :]
            return y + jnp.dot(lhs.astype(jnp.bfloat16), wo_h, preferred_element_type=jnp.float32)

        if p == 0:
            wo_cp.wait()
        y = lax.fori_loop(0, hkv, head, jnp.zeros((8, d_model), jnp.float32))
        return jnp.broadcast_to(jnp.sum(y, axis=0, keepdims=True), (8, d_model))

    def ffn(p, xn):
        if p == 0:
            b1_cp.wait()
            w1_cp.wait()
            w2_cp.wait()
        h = jnp.dot(xn.astype(jnp.bfloat16), w1_s[...], preferred_element_type=jnp.float32)
        h = h + b1_s[...].astype(jnp.float32)
        sp = jnp.log1p(jnp.exp(-jnp.abs(h))) + jnp.where(h > 0, h, 0.0)
        act = h * jnp.tanh(sp)
        return jnp.dot(act.astype(jnp.bfloat16), w2_s[...], preferred_element_type=jnp.float32)

    x_cp.wait()
    x = jnp.broadcast_to(x_s[...].astype(jnp.float32), (8, d_model))
    for p in range(2):
        x = x + attention(p, _layernorm(x))
        x = x + ffn(p, _layernorm(x))
    o_ref[0] = x[0:1, :].astype(o_ref.dtype)


@jax.jit
def pallas_interleave_layers__gqa_block_cached__dense_activation_mish__decode_kernel(
    A_x: jax.Array,
    A_k_cache: jax.Array,
    A_v_cache: jax.Array,
    A_wq: jax.Array,
    A_wo: jax.Array,
    B_x: jax.Array,
    B_w1: jax.Array,
    B_b1: jax.Array,
    B_w2: jax.Array,
):
    del B_x
    _, hkv, sk, dh = A_k_cache.shape
    d_model = A_x.shape[-1]
    f = B_w1.shape[-1]
    hq_dh = A_wq.shape[-1]
    nb = sk // BK
    ncache_heads = hkv - 1
    bf16 = jnp.bfloat16

    def kern(*refs):
        return _kernel(*refs, hkv=hkv, nb=nb, ncache_heads=ncache_heads)

    hbm = pl.BlockSpec(memory_space=pltpu.HBM)
    return pl.pallas_call(
        kern,
        in_specs=[hbm] * 8,
        out_specs=pl.BlockSpec(memory_space=pltpu.VMEM),
        out_shape=jax.ShapeDtypeStruct(A_x.shape, A_x.dtype),
        scratch_shapes=[
            pltpu.VMEM((ncache_heads * nb + NRING, BK, dh), bf16),
            pltpu.VMEM((hkv, d_model, hq_dh // hkv), bf16),
            pltpu.VMEM((hq_dh, d_model), bf16),
            pltpu.VMEM((d_model, f), bf16),
            pltpu.VMEM((f, d_model), bf16),
            pltpu.VMEM((1, d_model), bf16),
            pltpu.VMEM((1, f), bf16),
            pltpu.SemaphoreType.DMA((NRING,)),
            pltpu.SemaphoreType.DMA((KDEPTH,)),
            pltpu.SemaphoreType.DMA((hkv,)),
            pltpu.SemaphoreType.DMA((5,)),
        ],
        compiler_params=pltpu.CompilerParams(vmem_limit_bytes=128 * 1024 * 1024),
    )(A_x.reshape(1, 1, d_model), A_k_cache, A_v_cache, A_wq, A_wo, B_w1,
      B_b1.reshape(1, f), B_w2)
```

```python
import functools
import jax
import jax.numpy as jnp
from jax import lax
import jax.experimental.pallas as pl
import jax.experimental.pallas.tpu as pltpu

LN_EPS = 1e-5
LOG2E = 1.4426950408889634
GRP = 128
PGRP = 104
M_LO = 0x00FF00FF
M_E = 0x7F007F00
M_C = 0x0F000F00
M_S = -0x7FFF8000


def _layernorm(x):
    m = jnp.mean(x, axis=-1, keepdims=True)
    d = x - m
    v = jnp.mean(d * d, axis=-1, keepdims=True)
    return d * lax.rsqrt(v + LN_EPS)


def _shr(x, n):
    return lax.shift_right_logical(x, jnp.int32(n)) if n else x


def _shl(x, n):
    return lax.shift_left(x, jnp.int32(n)) if n else x


def _pack(w, ew):
    h = GRP // 2
    lo = (w[:h] & M_LO) | _shl(w[h:] & M_LO, 8)
    c = ew - (w & M_E)
    qn = GRP // 4
    code = _shr(c[:qn], 8) | _shr(c[qn:2 * qn], 4) | c[2 * qn:3 * qn] | _shl(c[3 * qn:], 4)
    sg = None
    for i in range(16):
        b = _shr(w[8 * i:8 * i + 8] & M_S, 15 - i)
        sg = b if sg is None else sg | b
    return lo, code, sg


def _unpack(lo, code, sg, ew):
    low = jnp.concatenate([lo & M_LO, _shr(lo, 8) & M_LO], axis=0)
    c = jnp.concatenate([_shl(code, 8) & M_C, _shl(code, 4) & M_C, code & M_C, _shr(code, 4) & M_C], axis=0)
    s = jnp.concatenate([_shl(sg, 15 - i) & M_S for i in range(16)], axis=0)
    return low | (ew - c) | s


def _kernel(x_hbm, k_hbm, v_hbm, wq_hbm, wo_hbm, w1_hbm, b1_hbm, w2_hbm, o_ref,
            pk, raw, s_ref, wq_s, wo_s, w1_s, w2_s, x_s, b1_s, ok_ref, em_ref,
            v_sem, k_sem, wq_sem, w_sem,
            *, hkv, nb, BK, NK, NV, CHUNK, PRIO):
    nstep = hkv * nb
    d_model = x_s.shape[-1]
    dh = raw.shape[-1]
    rep = wq_s.shape[-1] // dh
    scale = LOG2E * dh ** -0.5
    ngrp = BK // 2 // GRP

    def start_blk(hbm, t, dst, sem):
        base = (t % nb) * BK
        for c in range(BK // CHUNK):
            r = c * CHUNK
            pltpu.make_async_copy(
                hbm.at[0, t // nb, pl.ds(pl.multiple_of(base + r, CHUNK), CHUNK)],
                dst.at[pl.ds(r, CHUNK)], sem).start(priority=PRIO[c % len(PRIO)])

    def wait_blk(dst, sem):
        pltpu.make_async_copy(v_hbm.at[0, 0, pl.ds(0, BK)], dst, sem).wait()

    NPRE = NK - 1

    def k_start(t):
        start_blk(k_hbm, t, raw.at[NV + t % NK], k_sem.at[t % NK])

    def k_wait(t):
        wait_blk(raw.at[NV + t % NK], k_sem.at[t % NK])

    fb = NV + (nstep - 1) % NK

    def p2_step(i):
        return jnp.where(i < NV, nstep - NV + i, jnp.where(i < nb, nstep - nb + i - NV, i - nb))

    def v_slot(n):
        i = n - nstep
        pre = jnp.logical_and(i >= NV, i < NV + NPRE)
        ring = jnp.where(i >= NV + NPRE, n - NPRE, n) % NV
        return jnp.where(pre, NV + (nstep - NK + (i - NV)) % NK, ring)

    def v_start(n, pred):
        i = n - nstep
        t = jnp.where(i < 0, n, p2_step(i))
        slot = v_slot(n)

        @pl.when(pred)
        def _():
            start_blk(v_hbm, t, raw.at[slot], v_sem.at[slot])

    def v_wait(n):
        slot = v_slot(n)
        wait_blk(raw.at[slot], v_sem.at[slot])

    def v_next(p, n):
        if p == 0:
            v_start(n + NV, n + NV < nstep)
        else:
            i = n - nstep
            in_ring = jnp.logical_or(i < NV, i >= NV + NPRE)
            nn = n + NV + jnp.where(i < NV, NPRE, 0)
            v_start(nn, jnp.logical_and(in_ring, nn < 2 * nstep))

    def fb_start(i):
        t = p2_step(jnp.minimum(i, nstep - 1))

        @pl.when(jnp.logical_and(i < nstep, ok_ref[t] == 0))
        def _():
            start_blk(k_hbm, t, raw.at[fb], k_sem.at[0])

    def wq_copy(h):
        return pltpu.make_async_copy(wq_hbm.at[:, pl.ds(h * rep * dh, rep * dh)],
                                     wq_s.at[h], wq_sem.at[h])

    x_cp = pltpu.make_async_copy(x_hbm.at[0], x_s, w_sem.at[0])
    b1_cp = pltpu.make_async_copy(b1_hbm, b1_s, w_sem.at[1])
    wo_cp = pltpu.make_async_copy(wo_hbm, wo_s, w_sem.at[2])
    w1_cp = pltpu.make_async_copy(w1_hbm, w1_s, w_sem.at[3])
    w2_cp = pltpu.make_async_copy(w2_hbm, w2_s, w_sem.at[4])

    x_cp.start()
    wq_copy(0).start()
    for t in range(max(NK, NV)):
        if t < NK:
            k_start(t)
        if t < NV:
            v_start(t, True)
        if t == min(NK, max(NK, NV) - 1):
            for h in range(1, hkv):
                wq_copy(h).start()
            b1_cp.start()
            wo_cp.start()

    row = lax.broadcasted_iota(jnp.int32, (8, dh), 0)

    def qk(q, kb):
        return lax.dot_general(q, kb, (((1,), (1,)), ((), ())), preferred_element_type=jnp.float32)

    def qk_and_pack(q, t, slot):
        mx = jnp.zeros((8, dh), jnp.float32)
        ss = []
        for g in range(ngrp):
            kb = raw[NV + slot, pl.ds(2 * GRP * g, 2 * GRP), :]
            ss.append(qk(q, kb))
            w = pltpu.bitcast(kb, jnp.int32)
            e = w & M_E
            e = jnp.maximum(lax.bitcast_convert_type(e, jnp.float32),
                            lax.bitcast_convert_type(_shl(e, 16), jnp.float32))
            for i in range(GRP // 8):
                mx = jnp.maximum(mx, e[8 * i:8 * i + 8])
        mx = jnp.max(jnp.max(mx, axis=0, keepdims=True), axis=1, keepdims=True)
        em = jnp.max(_shr(lax.bitcast_convert_type(mx, jnp.int32), 24))
        ew = em * 0x01000100
        bad = jnp.zeros((8, dh), jnp.int32)
        for g in range(ngrp):
            w = pltpu.bitcast(raw[NV + slot, pl.ds(2 * GRP * g, 2 * GRP), :], jnp.int32)
            lo, code, sg = _pack(w, ew)
            r0 = g * PGRP
            pk[t, pl.ds(r0, GRP // 2), :] = lo
            pk[t, pl.ds(r0 + GRP // 2, GRP // 4), :] = code
            pk[t, pl.ds(r0 + 3 * GRP // 4, 8), :] = sg
            d = _unpack(lo, code, sg, ew) ^ w
            for i in range(GRP // 8):
                bad = bad | d[8 * i:8 * i + 8]
        nbad = jnp.max(jnp.where(bad != 0, 1.0, 0.0))
        ok_ref[t] = jnp.where(nbad > 0, 0, 1).astype(jnp.int32)
        em_ref[t] = ew
        return jnp.concatenate(ss, axis=1)

    def qk_packed(q, t):
        ew = em_ref[t]
        for g in range(ngrp):
            r0 = g * PGRP
            lo = pk[t, pl.ds(r0, GRP // 2), :]
            code = pk[t, pl.ds(r0 + GRP // 2, GRP // 4), :]
            sg = pk[t, pl.ds(r0 + 3 * GRP // 4, 8), :]
            kb = pltpu.bitcast(_unpack(lo, code, sg, ew), jnp.bfloat16)
            s_ref[:, pl.ds(2 * GRP * g, 2 * GRP)] = qk(q, kb)

    def attention(p, xn):
        xn_b = xn.astype(jnp.bfloat16)

        def head(hi, y):
            h = hi if p == 0 else (hi + hkv - 1) % hkv
            if p == 0:
                wq_copy(h).wait()
            qf = jnp.dot(xn_b, wq_s[h], preferred_element_type=jnp.float32)
            q = jnp.zeros((8, dh), jnp.float32)
            for r in range(rep):
                q = jnp.where(row == r, qf[:, r * dh:(r + 1) * dh], q)
            q = q.astype(jnp.bfloat16)

            def step(j, carry):
                m, l, acc = carry
                i = hi * nb + j
                if p == 0:
                    t = i
                    k_wait(t)
                    s = qk_and_pack(q, t, t % NK)

                    @pl.when(t + NK < nstep)
                    def _():
                        k_start(t + NK)

                    @pl.when(t + NK == nstep - 1)
                    def _():
                        w1_cp.start()
                        w2_cp.start()

                    v_start(nstep + NV + t - (nstep - NK),
                            jnp.logical_and(t >= nstep - NK, t < nstep - NK + NPRE))
                else:
                    t = p2_step(i)
                    ok = ok_ref[t] != 0

                    @pl.when(ok)
                    def _():
                        qk_packed(q, t)

                    @pl.when(jnp.logical_not(ok))
                    def _():
                        wait_blk(raw.at[fb], k_sem.at[0])
                        s_ref[...] = qk(q, raw[fb])

                    fb_start(i + 1)
                    s = s_ref[...]
                n = p * nstep + i
                m_new = jnp.maximum(m, jnp.max(s, axis=-1, keepdims=True))
                alpha = jnp.exp2((m - m_new) * scale)
                pr = jnp.exp2((s - m_new) * scale)
                l = alpha * l + jnp.sum(pr, axis=-1, keepdims=True)
                if p == 0:
                    v_wait(n)
                else:
                    @pl.when(i >= NV)
                    def _():
                        v_wait(n)
                pv = jnp.dot(pr.astype(jnp.bfloat16), raw[v_slot(n)], preferred_element_type=jnp.float32)
                acc = alpha * acc + pv
                v_next(p, n)
                return m_new, l, acc

            init = (jnp.full((8, 1), -1e30, jnp.float32), jnp.zeros((8, 1), jnp.float32),
                    jnp.zeros((8, dh), jnp.float32))
            _, l, acc = lax.fori_loop(0, nb, step, init)
            o = acc / l
            lhs = jnp.concatenate([jnp.where(row == r, o, 0.0) for r in range(rep)], axis=1)
            wo_h = wo_s[pl.ds(pl.multiple_of(h * rep * dh, rep * dh), rep * dh), :]
            return y + jnp.dot(lhs.astype(jnp.bfloat16), wo_h, preferred_element_type=jnp.float32)

        if p == 0:
            wo_cp.wait()
        else:
            fb_start(0)
        y = lax.fori_loop(0, hkv, head, jnp.zeros((8, d_model), jnp.float32))
        return jnp.broadcast_to(jnp.sum(y, axis=0, keepdims=True), (8, d_model))

    def ffn(p, xn):
        if p == 0:
            w1_cp.wait()
        h = jnp.dot(xn.astype(jnp.bfloat16), w1_s[...], preferred_element_type=jnp.float32)
        h = h + b1v
        sp = jnp.log1p(jnp.exp(-jnp.abs(h))) + jnp.where(h > 0, h, 0.0)
        act = h * jnp.tanh(sp)
        if p == 0:
            w2_cp.wait()
        return jnp.dot(act.astype(jnp.bfloat16), w2_s[...], preferred_element_type=jnp.float32)

    x_cp.wait()
    x = jnp.broadcast_to(x_s[...].astype(jnp.float32), (8, d_model))
    b1_cp.wait()
    b1v = b1_s[...].astype(jnp.float32).reshape(1, -1)
    for p in range(2):
        x = x + attention(p, _layernorm(x))
        x = x + ffn(p, _layernorm(x))
    o_ref[0] = x[0:1, :].astype(o_ref.dtype)


def build(BK=4096, NK=4, NV=8, CHUNK=128, PRIO=(0, 1, 1, 1, 1)):
    @jax.jit
    def fn(A_x, A_k_cache, A_v_cache, A_wq, A_wo, B_x, B_w1, B_b1, B_w2):
        del B_x
        _, hkv, sk, dh = A_k_cache.shape
        d_model = A_x.shape[-1]
        f = B_w1.shape[-1]
        hq_dh = A_wq.shape[-1]
        nb = sk // BK
        bf16 = jnp.bfloat16
        kern = functools.partial(_kernel, hkv=hkv, nb=nb, BK=BK, NK=NK, NV=NV, CHUNK=CHUNK, PRIO=PRIO)
        hbm = pl.BlockSpec(memory_space=pltpu.HBM)
        return pl.pallas_call(
            kern,
            in_specs=[hbm] * 8,
            out_specs=pl.BlockSpec(memory_space=pltpu.VMEM),
            out_shape=jax.ShapeDtypeStruct(A_x.shape, A_x.dtype),
            scratch_shapes=[
                pltpu.VMEM((hkv * nb, BK // 2 // GRP * PGRP, dh), jnp.int32),
                pltpu.VMEM((NV + NK, BK, dh), bf16),
                pltpu.VMEM((8, BK), jnp.float32),
                pltpu.VMEM((hkv, d_model, hq_dh // hkv), bf16),
                pltpu.VMEM((hq_dh, d_model), bf16),
                pltpu.VMEM((d_model, f), bf16),
                pltpu.VMEM((f, d_model), bf16),
                pltpu.VMEM((1, d_model), bf16),
                pltpu.VMEM((f,), bf16),
                pltpu.SMEM((hkv * nb,), jnp.int32),
                pltpu.SMEM((hkv * nb,), jnp.int32),
                pltpu.SemaphoreType.DMA((NV + NK,)),
                pltpu.SemaphoreType.DMA((NK,)),
                pltpu.SemaphoreType.DMA((hkv,)),
                pltpu.SemaphoreType.DMA((5,)),
            ],
            compiler_params=pltpu.CompilerParams(vmem_limit_bytes=128 * 1024 * 1024,
                                                 disable_bounds_checks=True),
        )(A_x, A_k_cache, A_v_cache, A_wq, A_wo, B_w1, B_b1, B_w2)
    return fn


pallas_interleave_layers__gqa_block_cached__dense_activation_mish__decode_kernel = build()
```
